```python
import os as _os
_os.environ.setdefault("JAX_PLATFORMS", "cpu")
import jax
import jax.numpy as jnp

def _softmax(x, axis=-1):
    return jax.nn.softmax(x, axis=axis)
def _gelu(x):
    return jax.nn.gelu(x, approximate=True)
def _silu(x):
    return jax.nn.silu(x)
def _sigmoid(x):
    return jax.nn.sigmoid(x)
def _layernorm(x, axis=-1, eps=1e-5):
    m = jnp.mean(x, axis=axis, keepdims=True)
    v = jnp.var(x, axis=axis, keepdims=True)
    return (x - m) / jnp.sqrt(v + eps)
def _scatter_add(tgt, idx, src, axis=0):
    return tgt.at[idx].add(src)
def _segment_sum(src, seg, n):
    return jax.ops.segment_sum(src, seg, n)
class _Rng:
    def __init__(self, key):
        self._k = key
    def _next(self):
        self._k, sub = jax.random.split(self._k)
        return sub
    def normal(self, shape):
        return jax.random.normal(self._next(), shape, dtype=jnp.bfloat16)
    def randint(self, lo, hi, shape):
        return jax.random.randint(self._next(), shape, lo, hi, dtype=jnp.int32)
    def uniform(self, shape, lo=0.0, hi=1.0):
        return jax.random.uniform(self._next(), shape, jnp.bfloat16, lo, hi)
    def permutation(self, n):
        return jax.random.permutation(self._next(), n)


kernel_name = 'sequential_preLN__spectral_gfnet__glu_gated_bilinear__prompt'

def setup_inputs():
    _rng = _Rng(jax.random.key(int.from_bytes(__import__("os").urandom(4), "little")))
    _w = (lambda a: (lambda t: t.astype(jnp.bfloat16) if jnp.issubdtype(t.dtype, jnp.floating) else t)(jnp.asarray(a)))
    def _A_setup():
        B, S, D = 1, 2048, 448
        Df = D // 2 + 1
        return {
            "x": _w((lambda *s: _rng.normal(s) * 0.05)(B, S, D)),
            "w_r": _w((lambda *s: _rng.normal(s) * 0.2)(S, Df) * 0.02),
            "w_i": _w((lambda *s: _rng.normal(s) * 0.2)(S, Df) * 0.02),
        }
    _A_in = _A_setup()

    def _B_setup():
        B, S, D, F = 1, 2048, 448, 1792
        return {
            "x": _w((lambda *s: _rng.normal(s) * 0.05)(B, S, D)),
            "w_gate": _w((lambda *s: _rng.normal(s) * 0.05)(D, F) * (D ** -0.5)),
            "w_up": _w((lambda *s: _rng.normal(s) * 0.05)(D, F) * (D ** -0.5)),
            "w_down": _w((lambda *s: _rng.normal(s) * 0.05)(F, D) * (F ** -0.5)),
        }
    _B_in = _B_setup()

    return {
        "A_x": _A_in["x"],
        "A_w_r": _A_in["w_r"],
        "A_w_i": _A_in["w_i"],
        "B_x": _B_in["x"],
        "B_w_gate": _B_in["w_gate"],
        "B_w_up": _B_in["w_up"],
        "B_w_down": _B_in["w_down"],
    }

def reference(A_x, A_w_r, A_w_i, B_x, B_w_gate, B_w_up, B_w_down):
    def _A_ref(x, w_r, w_i):
        B, S, D = x.shape
        X = (lambda x, axes=(-2,-1): jnp.fft.rfft2(x.astype(jnp.float32), axes=axes))(x, axes=(-2, -1))
        W = w_r + 1j * w_i
        X = X * W
        y = (lambda x, s, axes=(-2,-1): jnp.fft.irfft2(x, s=s, axes=axes).astype(jnp.bfloat16))(X, (S, D), axes=(-2, -1))
        return y

    def _B_ref(x, w_gate, w_up, w_down):
        g = jnp.einsum("bsd,df->bsf", x, w_gate)
        u = jnp.einsum("bsd,df->bsf", x, w_up)
        h = g * u
        return jnp.einsum("bsf,fd->bsd", h, w_down)

    x = A_x
    h = x + _A_ref(_layernorm(x, axis=-1), A_w_r, A_w_i)
    h2 = h + _B_ref(_layernorm(h, axis=-1), B_w_gate, B_w_up, B_w_down)
    return h2
```

```python
import functools
import math

import numpy as np
import jax
import jax.numpy as jnp
from jax import lax
import jax.experimental.pallas as pl
import jax.experimental.pallas.tpu as pltpu

S = 2048
D = 448
DF = D // 2 + 1
FP = 256
F = 1792
N1 = 16
N2 = 128
TM = 256
EPS = 1e-5


def _constants():
    d = np.arange(D)[:, None].astype(np.float64)
    k = np.arange(DF)[None, :].astype(np.float64)
    ang = 2.0 * np.pi * d * k / D
    md = np.zeros((D, 2 * FP), np.float64)
    md[:, :DF] = np.cos(ang)
    md[:, FP:FP + DF] = -np.sin(ang)
    ck = np.full((DF,), 2.0)
    ck[0] = 1.0
    ck[DF - 1] = 1.0
    mi = np.zeros((2 * FP, D), np.float64)
    mi[:DF, :] = (ck[:, None] * np.cos(ang.T)) / (S * D)
    mi[FP:FP + DF, :] = -(ck[:, None] * np.sin(ang.T)) / (S * D)
    n1 = np.arange(N1)[:, None, None].astype(np.float64)
    k2 = np.arange(N2)[None, :, None].astype(np.float64)
    n2 = np.arange(N2)[None, None, :].astype(np.float64)
    th = 2.0 * np.pi * k2 * (n1 + N1 * n2) / S
    gf = np.concatenate([np.cos(th), -np.sin(th)], axis=1)
    tht = np.transpose(th, (0, 2, 1))
    gi = np.concatenate([np.cos(tht), np.sin(tht)], axis=1)
    return (md.astype(np.float32), mi.astype(np.float32),
            gf.astype(np.float32), gi.astype(np.float32))


def _fft4(x0, x1, x2, x3, sign):
    s02 = (x0[0] + x2[0], x0[1] + x2[1])
    d02 = (x0[0] - x2[0], x0[1] - x2[1])
    s13 = (x1[0] + x3[0], x1[1] + x3[1])
    d13 = (x1[0] - x3[0], x1[1] - x3[1])
    y0 = (s02[0] + s13[0], s02[1] + s13[1])
    y2 = (s02[0] - s13[0], s02[1] - s13[1])
    if sign < 0:
        y1 = (d02[0] + d13[1], d02[1] - d13[0])
        y3 = (d02[0] - d13[1], d02[1] + d13[0])
    else:
        y1 = (d02[0] - d13[1], d02[1] + d13[0])
        y3 = (d02[0] + d13[1], d02[1] - d13[0])
    return y0, y1, y2, y3


def _twiddle(z, p, sign):
    p = p % 16
    if p == 0:
        return z
    zr, zi = z
    if p == 4:
        return (-zi, zr) if sign > 0 else (zi, -zr)
    c = math.cos(2.0 * math.pi * p / 16.0)
    s = sign * math.sin(2.0 * math.pi * p / 16.0)
    return (zr * c - zi * s, zr * s + zi * c)


def _fft16(xs, sign):
    t = [None] * 16
    for b in range(4):
        y = _fft4(xs[b], xs[4 + b], xs[8 + b], xs[12 + b], sign)
        for c in range(4):
            t[b * 4 + c] = _twiddle(y[c], b * c, sign)
    out = [None] * 16
    for c in range(4):
        y = _fft4(t[c], t[4 + c], t[8 + c], t[12 + c], sign)
        for e in range(4):
            out[c + 4 * e] = y[e]
    return out


def _layernorm(xf):
    m = jnp.mean(xf, axis=-1, keepdims=True)
    xc = xf - m
    v = jnp.mean(xc * xc, axis=-1, keepdims=True)
    return xc * lax.rsqrt(v + EPS)


def _kernel(x_ref, wr_ref, wi_ref, wg_ref, wu_ref, wd_ref,
            md_ref, mi_ref, gf_ref, gi_ref, o_ref, a_ref, b_ref):
    step = pl.program_id(0)

    @pl.when(step == 0)
    def _spectral():
        RC = 256

        def p1(i, carry):
            r = pl.multiple_of(i * RC, RC)
            xn = _layernorm(x_ref[pl.ds(r, RC), :].astype(jnp.float32))
            a = jnp.dot(xn.astype(jnp.bfloat16), md_ref[...],
                        preferred_element_type=jnp.float32)
            for c in range(4):
                a_ref[c, pl.ds(r, RC), :] = a[:, c * 128:(c + 1) * 128]
            return carry

        lax.fori_loop(0, S // RC, p1, 0)

        def p2(n1, carry):
            yb = jnp.concatenate(
                [a_ref[c, pl.ds(n1, N2, stride=N1), :] for c in range(4)],
                axis=1).astype(jnp.bfloat16)
            pq = jnp.dot(gf_ref[n1], yb, preferred_element_type=jnp.float32)
            r = pl.multiple_of(n1 * N2, N2)
            b_ref[pl.ds(r, N2), :FP] = pq[:N2, :FP] - pq[N2:, FP:]
            b_ref[pl.ds(r, N2), FP:] = pq[:N2, FP:] + pq[N2:, :FP]
            return carry

        lax.fori_loop(0, N1, p2, 0)

        R3 = 8

        def p3(i, carry):
            r = i * R3
            for lc in range(2):
                lo = lc * 128
                xs = [(b_ref[pl.ds(n * N2 + r, R3), lo:lo + 128],
                       b_ref[pl.ds(n * N2 + r, R3), FP + lo:FP + lo + 128])
                      for n in range(N1)]
                xk = _fft16(xs, -1)
                zs = []
                for k1 in range(N1):
                    wr = wr_ref[pl.ds(k1 * N2 + r, R3), lo:lo + 128].astype(jnp.float32)
                    wi = wi_ref[pl.ds(k1 * N2 + r, R3), lo:lo + 128].astype(jnp.float32)
                    zr, zi = xk[k1]
                    zs.append((zr * wr - zi * wi, zr * wi + zi * wr))
                us = _fft16(zs, +1)
                for n in range(N1):
                    b_ref[pl.ds(n * N2 + r, R3), lo:lo + 128] = us[n][0]
                    b_ref[pl.ds(n * N2 + r, R3), FP + lo:FP + lo + 128] = us[n][1]
            return carry

        lax.fori_loop(0, N2 // R3, p3, 0)

        def p4(n1, carry):
            r = pl.multiple_of(n1 * N2, N2)
            ub = b_ref[pl.ds(r, N2), :].astype(jnp.bfloat16)
            pq = jnp.dot(gi_ref[n1], ub, preferred_element_type=jnp.float32)
            vr = pq[:N2, :FP] - pq[N2:, FP:]
            vi = pq[:N2, FP:] + pq[N2:, :FP]
            a_ref[0, pl.ds(n1, N2, stride=N1), :] = vr[:, :128]
            a_ref[1, pl.ds(n1, N2, stride=N1), :] = vr[:, 128:]
            a_ref[2, pl.ds(n1, N2, stride=N1), :] = vi[:, :128]
            a_ref[3, pl.ds(n1, N2, stride=N1), :] = vi[:, 128:]
            return carry

        lax.fori_loop(0, N1, p4, 0)

    r0 = pl.multiple_of(step * TM, TM)
    yp = jnp.concatenate([a_ref[c, pl.ds(r0, TM), :] for c in range(4)],
                         axis=1).astype(jnp.bfloat16)
    y = jnp.dot(yp, mi_ref[...], preferred_element_type=jnp.float32)
    h = x_ref[pl.ds(r0, TM), :] + y.astype(jnp.bfloat16)
    hf = h.astype(jnp.float32)
    hn = _layernorm(hf).astype(jnp.bfloat16)
    g = jnp.dot(hn, wg_ref[...], preferred_element_type=jnp.float32)
    u = jnp.dot(hn, wu_ref[...], preferred_element_type=jnp.float32)
    gu = (g * u).astype(jnp.bfloat16)
    dn = jnp.dot(gu, wd_ref[...], preferred_element_type=jnp.float32)
    o_ref[...] = (hf + dn).astype(o_ref.dtype)


@jax.jit
def pallas_sequential_preLN__spectral_gfnet__glu_gated_bilinear__prompt_kernel(
    A_x: jax.Array,
    A_w_r: jax.Array,
    A_w_i: jax.Array,
    B_x: jax.Array,
    B_w_gate: jax.Array,
    B_w_up: jax.Array,
    B_w_down: jax.Array,
):
    x = A_x.reshape(S, D)
    wr = jnp.pad(A_w_r, ((0, 0), (0, FP - DF)))
    wi = jnp.pad(A_w_i, ((0, 0), (0, FP - DF)))
    md, mi, gf, gi = [jnp.asarray(c, dtype=jnp.bfloat16) for c in _constants()]

    full = lambda shape: pl.BlockSpec(shape, lambda i: (0,) * len(shape))
    out = pl.pallas_call(
        _kernel,
        grid=(S // TM,),
        in_specs=[
            full((S, D)), full((S, FP)), full((S, FP)),
            full((D, F)), full((D, F)), full((F, D)),
            full((D, 2 * FP)), full((2 * FP, D)),
            full((N1, 2 * N2, N2)), full((N1, 2 * N2, N2)),
        ],
        out_specs=pl.BlockSpec((TM, D), lambda i: (i, 0)),
        out_shape=jax.ShapeDtypeStruct((S, D), jnp.bfloat16),
        scratch_shapes=[
            pltpu.VMEM((4, S, 128), jnp.float32),
            pltpu.VMEM((S, 2 * FP), jnp.float32),
        ],
        compiler_params=pltpu.CompilerParams(
            dimension_semantics=("arbitrary",),
            vmem_limit_bytes=100 * 1024 * 1024,
        ),
    )(x, wr, wi, B_w_gate, B_w_up, B_w_down, md, mi, gf, gi)
    return out.reshape(1, S, D)
```

```python
import functools
import math

import numpy as np
import jax
import jax.numpy as jnp
from jax import lax
import jax.experimental.pallas as pl
import jax.experimental.pallas.tpu as pltpu

S = 2048
D = 448
DF = D // 2 + 1
FP = 256
F = 1792
N1 = 16
N2 = 128
TM = 512
EPS = 1e-5


def _constants():
    d = np.arange(D)[:, None].astype(np.float64)
    k = np.arange(DF)[None, :].astype(np.float64)
    ang = 2.0 * np.pi * d * k / D
    md = np.zeros((D, 2 * FP), np.float64)
    md[:, :DF] = np.cos(ang)
    md[:, FP:FP + DF] = -np.sin(ang)
    ck = np.full((DF,), 2.0)
    ck[0] = 1.0
    ck[DF - 1] = 1.0
    mi = np.zeros((2 * FP, D), np.float64)
    mi[:DF, :] = (ck[:, None] * np.cos(ang.T)) / (S * D)
    mi[FP:FP + DF, :] = -(ck[:, None] * np.sin(ang.T)) / (S * D)
    n1 = np.arange(N1)[:, None, None].astype(np.float64)
    k2 = np.arange(N2)[None, :, None].astype(np.float64)
    n2 = np.arange(N2)[None, None, :].astype(np.float64)
    th = 2.0 * np.pi * k2 * (n1 + N1 * n2) / S
    gf = np.concatenate([np.cos(th), -np.sin(th)], axis=1)
    tht = np.transpose(th, (0, 2, 1))
    gi = np.concatenate([np.cos(tht), np.sin(tht)], axis=1)
    return (md.astype(np.float32), mi.astype(np.float32),
            gf.astype(np.float32), gi.astype(np.float32))


def _fft4(x0, x1, x2, x3, sign):
    s02 = (x0[0] + x2[0], x0[1] + x2[1])
    d02 = (x0[0] - x2[0], x0[1] - x2[1])
    s13 = (x1[0] + x3[0], x1[1] + x3[1])
    d13 = (x1[0] - x3[0], x1[1] - x3[1])
    y0 = (s02[0] + s13[0], s02[1] + s13[1])
    y2 = (s02[0] - s13[0], s02[1] - s13[1])
    if sign < 0:
        y1 = (d02[0] + d13[1], d02[1] - d13[0])
        y3 = (d02[0] - d13[1], d02[1] + d13[0])
    else:
        y1 = (d02[0] - d13[1], d02[1] + d13[0])
        y3 = (d02[0] + d13[1], d02[1] - d13[0])
    return y0, y1, y2, y3


def _twiddle(z, p, sign):
    p = p % 16
    if p == 0:
        return z
    zr, zi = z
    if p == 4:
        return (-zi, zr) if sign > 0 else (zi, -zr)
    c = math.cos(2.0 * math.pi * p / 16.0)
    s = sign * math.sin(2.0 * math.pi * p / 16.0)
    return (zr * c - zi * s, zr * s + zi * c)


def _fft16(xs, sign):
    t = [None] * 16
    for b in range(4):
        y = _fft4(xs[b], xs[4 + b], xs[8 + b], xs[12 + b], sign)
        for c in range(4):
            t[b * 4 + c] = _twiddle(y[c], b * c, sign)
    out = [None] * 16
    for c in range(4):
        y = _fft4(t[c], t[4 + c], t[8 + c], t[12 + c], sign)
        for e in range(4):
            out[c + 4 * e] = y[e]
    return out


def _layernorm_t(xf):
    m = jnp.mean(xf, axis=0, keepdims=True)
    xc = xf - m
    v = jnp.mean(xc * xc, axis=0, keepdims=True)
    return xc * lax.rsqrt(v + EPS)


_TN = (((0,), (0,)), ((), ()))
_NT = (((1,), (1,)), ((), ()))


def _kernel(x_ref, wr_ref, wi_ref, wg_ref, wu_ref, wd_ref,
            md_ref, mi_ref, gf_ref, gi_ref, o_ref, a_ref, b_ref):
    step = pl.program_id(0)

    @pl.when(step == 0)
    def _spectral():
        RC = 256

        def p1(i, carry):
            r = pl.multiple_of(i * RC, RC)
            xn = _layernorm_t(x_ref[:, pl.ds(r, RC)].astype(jnp.float32))
            a = lax.dot_general(xn.astype(jnp.bfloat16), md_ref[...], _TN,
                                preferred_element_type=jnp.float32)
            for c in range(4):
                a_ref[c, pl.ds(r, RC), :] = a[:, c * 128:(c + 1) * 128]
            return carry

        lax.fori_loop(0, S // RC, p1, 0)

        def p2(n1, carry):
            yb = jnp.concatenate(
                [a_ref[c, pl.ds(n1, N2, stride=N1), :] for c in range(4)],
                axis=1).astype(jnp.bfloat16)
            pq = jnp.dot(gf_ref[n1], yb, preferred_element_type=jnp.float32)
            r = pl.multiple_of(n1 * N2, N2)
            b_ref[pl.ds(r, N2), :FP] = pq[:N2, :FP] - pq[N2:, FP:]
            b_ref[pl.ds(r, N2), FP:] = pq[:N2, FP:] + pq[N2:, :FP]
            return carry

        lax.fori_loop(0, N1, p2, 0)

        R3 = 8

        def p3(i, carry):
            r = i * R3
            for lc in range(2):
                lo = lc * 128
                xs = [(b_ref[pl.ds(n * N2 + r, R3), lo:lo + 128],
                       b_ref[pl.ds(n * N2 + r, R3), FP + lo:FP + lo + 128])
                      for n in range(N1)]
                xk = _fft16(xs, -1)
                zs = []
                for k1 in range(N1):
                    wr = wr_ref[pl.ds(k1 * N2 + r, R3), lo:lo + 128].astype(jnp.float32)
                    wi = wi_ref[pl.ds(k1 * N2 + r, R3), lo:lo + 128].astype(jnp.float32)
                    zr, zi = xk[k1]
                    zs.append((zr * wr - zi * wi, zr * wi + zi * wr))
                us = _fft16(zs, +1)
                for n in range(N1):
                    b_ref[pl.ds(n * N2 + r, R3), lo:lo + 128] = us[n][0]
                    b_ref[pl.ds(n * N2 + r, R3), FP + lo:FP + lo + 128] = us[n][1]
            return carry

        lax.fori_loop(0, N2 // R3, p3, 0)

        def p4(n1, carry):
            r = pl.multiple_of(n1 * N2, N2)
            ub = b_ref[pl.ds(r, N2), :].astype(jnp.bfloat16)
            pq = jnp.dot(gi_ref[n1], ub, preferred_element_type=jnp.float32)
            vr = pq[:N2, :FP] - pq[N2:, FP:]
            vi = pq[:N2, FP:] + pq[N2:, :FP]
            a_ref[0, pl.ds(n1, N2, stride=N1), :] = vr[:, :128]
            a_ref[1, pl.ds(n1, N2, stride=N1), :] = vr[:, 128:]
            a_ref[2, pl.ds(n1, N2, stride=N1), :] = vi[:, :128]
            a_ref[3, pl.ds(n1, N2, stride=N1), :] = vi[:, 128:]
            return carry

        lax.fori_loop(0, N1, p4, 0)

    r0 = pl.multiple_of(step * TM, TM)
    yp = jnp.concatenate([a_ref[c, pl.ds(r0, TM), :] for c in range(4)],
                         axis=1).astype(jnp.bfloat16)
    yt = lax.dot_general(mi_ref[...], yp, _NT, preferred_element_type=jnp.float32)
    ht = x_ref[:, pl.ds(r0, TM)] + yt.astype(jnp.bfloat16)
    hf = ht.astype(jnp.float32)
    hn = _layernorm_t(hf).astype(jnp.bfloat16)
    g = lax.dot_general(hn, wg_ref[...], _TN, preferred_element_type=jnp.float32)
    u = lax.dot_general(hn, wu_ref[...], _TN, preferred_element_type=jnp.float32)
    gu = (g * u).astype(jnp.bfloat16)
    dn = lax.dot_general(wd_ref[...], gu, _NT, preferred_element_type=jnp.float32)
    o_ref[...] = (hf + dn).astype(o_ref.dtype)


@jax.jit
def pallas_sequential_preLN__spectral_gfnet__glu_gated_bilinear__prompt_kernel(
    A_x: jax.Array,
    A_w_r: jax.Array,
    A_w_i: jax.Array,
    B_x: jax.Array,
    B_w_gate: jax.Array,
    B_w_up: jax.Array,
    B_w_down: jax.Array,
):
    x = A_x.reshape(S, D).T
    wr = jnp.pad(A_w_r, ((0, 0), (0, FP - DF)))
    wi = jnp.pad(A_w_i, ((0, 0), (0, FP - DF)))
    md, mi, gf, gi = [jnp.asarray(c, dtype=jnp.bfloat16) for c in _constants()]
    mi = mi.T

    full = lambda shape: pl.BlockSpec(shape, lambda i: (0,) * len(shape))
    out = pl.pallas_call(
        _kernel,
        grid=(S // TM,),
        in_specs=[
            full((D, S)), full((S, FP)), full((S, FP)),
            full((D, F)), full((D, F)), full((D, F)),
            full((D, 2 * FP)), full((D, 2 * FP)),
            full((N1, 2 * N2, N2)), full((N1, 2 * N2, N2)),
        ],
        out_specs=pl.BlockSpec((D, TM), lambda i: (0, i)),
        out_shape=jax.ShapeDtypeStruct((D, S), jnp.bfloat16),
        scratch_shapes=[
            pltpu.VMEM((4, S, 128), jnp.float32),
            pltpu.VMEM((S, 2 * FP), jnp.float32),
        ],
        compiler_params=pltpu.CompilerParams(
            dimension_semantics=("arbitrary",),
            vmem_limit_bytes=100 * 1024 * 1024,
        ),
    )(x, wr, wi, B_w_gate, B_w_up, B_w_down.T, md, mi, gf, gi)
    return out.T.reshape(1, S, D)
```
